```python
import jax
import jax.numpy as jnp

def _softmax(x, axis=-1):
    return jax.nn.softmax(x, axis=axis)
def _gelu(x):
    return jax.nn.gelu(x, approximate=True)
def _silu(x):
    return jax.nn.silu(x)
def _sigmoid(x):
    return jax.nn.sigmoid(x)
def _layernorm(x, axis=-1, eps=1e-5):
    m = jnp.mean(x, axis=axis, keepdims=True)
    v = jnp.var(x, axis=axis, keepdims=True)
    return (x - m) / jnp.sqrt(v + eps)
def _scatter_add(tgt, idx, src, axis=0):
    return tgt.at[idx].add(src)
def _segment_sum(src, seg, n):
    return jax.ops.segment_sum(src, seg, n)
class _Rng:
    def __init__(self, key):
        self._k = key
    def _next(self):
        self._k, sub = jax.random.split(self._k)
        return sub
    def normal(self, shape):
        return jax.random.normal(self._next(), shape, dtype=jnp.bfloat16)
    def randint(self, lo, hi, shape):
        return jax.random.randint(self._next(), shape, lo, hi, dtype=jnp.int32)
    def uniform(self, shape, lo=0.0, hi=1.0):
        return jax.random.uniform(self._next(), shape, jnp.bfloat16, lo, hi)
    def permutation(self, n):
        return jax.random.permutation(self._next(), n)


kernel_name = 'gated_mix__compressed_kv_cla__sliding_local_dilated__prompt'

def setup_inputs():
    _rng = _Rng(jax.random.key(int.from_bytes(__import__("os").urandom(4), "little")))
    _w = (lambda a: (lambda t: t.astype(jnp.bfloat16) if jnp.issubdtype(t.dtype, jnp.floating) else t)(jnp.asarray(a)))
    def _A_setup():
        B, H, Sq, Sk, D, M = 1, 32, 2048, 2048, 128, 1024
        Dc = 4 * D
        return {
            "x": _w((lambda *s: _rng.normal(s) * 0.05)(B, Sq, M)),
            "c_kv": _w((lambda *s: _rng.normal(s) * 0.05)(B, Sk, Dc)),
            "w_q": _w((lambda *s: _rng.normal(s) * 0.05)(M, H, D) * (M ** -0.5)),
            "w_uk": _w((lambda *s: _rng.normal(s) * 0.05)(Dc, H, D) * (Dc ** -0.5)),
            "w_uv": _w((lambda *s: _rng.normal(s) * 0.05)(Dc, H, D) * (Dc ** -0.5)),
            "w_o": _w((lambda *s: _rng.normal(s) * 0.05)(H, D, M) * ((H * D) ** -0.5)),
        }
    _A_in = _A_setup()

    def _B_setup():
        B, S, D = 1, 2048, 1024
        return {
            "x": _w((lambda *s: _rng.normal(s) * 0.05)(B, S, D)),
            "wqkv": _w((lambda *s: _rng.normal(s) * 0.05)(D, 3 * D)),
            "wo": _w((lambda *s: _rng.normal(s) * 0.05)(D, D)),
        }
    _B_in = _B_setup()

    return {
        "A_x": _A_in["x"],
        "A_c_kv": _A_in["c_kv"],
        "A_w_q": _A_in["w_q"],
        "A_w_uk": _A_in["w_uk"],
        "A_w_uv": _A_in["w_uv"],
        "A_w_o": _A_in["w_o"],
        "B_x": _B_in["x"],
        "B_wqkv": _B_in["wqkv"],
        "B_wo": _B_in["wo"],
        "gate_w": _w((lambda *s: _rng.normal(s) * 0.05)(1024)),
    }

def reference(A_x, A_c_kv, A_w_q, A_w_uk, A_w_uv, A_w_o, B_x, B_wqkv, B_wo, gate_w):
    def _A_ref(x, c_kv, w_q, w_uk, w_uv, w_o):
        B, Sq, M = x.shape[0], x.shape[1], x.shape[2]
        Sk = c_kv.shape[1]
        H, D = w_q.shape[1], w_q.shape[2]
        q = jnp.einsum("bqm,mhd->bhqd", x, w_q)
        k = jnp.einsum("bkc,chd->bhkd", c_kv, w_uk)
        v = jnp.einsum("bkc,chd->bhkd", c_kv, w_uv)
        scores = jnp.einsum("bhqd,bhkd->bhqk", q, k) * (D ** -0.5)
        off = Sk - Sq
        qi = jnp.arange(Sq)[:, None]
        kj = jnp.arange(Sk)[None, :]
        cmask = kj <= (qi + off)
        scores = jnp.where(cmask[None, None], scores, -1e9)
        p = _softmax(scores, axis=-1)
        ctx = jnp.einsum("bhqk,bhkd->bhqd", p, v)
        return jnp.einsum("bhqd,hdm->bqm", ctx, w_o)

    def _B_ref(x, wqkv, wo):
        B, S, D = x.shape
        H = 32; Dh = D // H
        W, dil = 8, 2
        qkv = (lambda x, *d: x.transpose(*d))((x @ wqkv).reshape(B, S, 3, H, Dh), 2, 0, 3, 1, 4)
        q, k, v = qkv[0], qkv[1], qkv[2]
        scale = Dh ** -0.5
        pos = jnp.arange(S)
        off = jnp.arange(W) * dil
        idx = pos[:, None] - off[None, :]
        mask = idx >= 0
        idx_c = jnp.where(mask, idx, 0).reshape(-1)
        kg = k[:, :, idx_c, :].reshape(B, H, S, W, Dh)
        vg = v[:, :, idx_c, :].reshape(B, H, S, W, Dh)
        logits = jnp.einsum("bhsd,bhswd->bhsw", q, kg) * scale
        logits = jnp.where(mask[None, None, :, :], logits, -1e9)
        attn = _softmax(logits, axis=-1)
        o = jnp.einsum("bhsw,bhswd->bhsd", attn, vg)
        return (lambda x, *d: x.transpose(*d))(o, 0, 2, 1, 3).reshape(B, S, D) @ wo

    x = A_x
    g = _sigmoid((x * gate_w).sum(-1, keepdims=True))
    a = _A_ref(x, A_c_kv, A_w_q, A_w_uk, A_w_uv, A_w_o)
    b = _B_ref(x, B_wqkv, B_wo)
    return g * a + (1 - g) * b
```

```python
import functools
import jax
import jax.numpy as jnp
import numpy as np
import jax.experimental.pallas as pl
import jax.experimental.pallas.tpu as pltpu

S, M, H, D, DC = 2048, 1024, 32, 128, 512
BQ = 256
RB = 256
NR = S // RB
HALO = 16
LOG2E = 1.4426950408889634
NEG = -1e30
F32, BF16, U32 = jnp.float32, jnp.bfloat16, jnp.uint32
DIAG_SPLIT = True


def _dot(a, b):
    return jnp.dot(a, b, preferred_element_type=F32)


def _dot_nt(a, b):
    return jax.lax.dot_general(a, b, (((1,), (1,)), ((), ())), preferred_element_type=F32)


def _head_weight(w_ref, h):
    w32 = w_ref[h // 2]
    sh = ((1 - h % 2) * 16).astype(U32)
    bits = (w32 << sh) & jnp.uint32(0xFFFF0000)
    return jax.lax.bitcast_convert_type(bits, F32).astype(BF16)


def _kernel(x_hbm, c_hbm, wq_hbm, wuk_hbm, wuv_hbm, wo_hbm, wqkv_hbm, wob_hbm, gw_ref, out_ref,
            x_ref, c_ref, wq_ref, wuk_ref, wuv_ref, wo_ref, wqkv_ref, wob_ref,
            ctx_ref, acc_ref, g_ref, kb_ref, vb_ref, xsem, sems):
    i = pl.program_id(0)

    def x_copy(r):
        return pltpu.make_async_copy(x_hbm.at[pl.ds(r * RB, RB), :], x_ref.at[pl.ds(r * RB, RB), :], xsem.at[r])

    def cp(n):
        src, dst = ((wqkv_hbm, wqkv_ref), (wob_hbm, wob_ref), (c_hbm, c_ref), (wo_hbm, wo_ref))[n]
        return pltpu.make_async_copy(src, dst, sems.at[n])

    def w_copies():
        return [pltpu.make_async_copy(src.bitcast(U32).at[:, j, :], dst.at[j], sems.at[4 + n])
                for j in range(H // 2)
                for n, (src, dst) in enumerate(((wq_hbm, wq_ref), (wuk_hbm, wuk_ref), (wuv_hbm, wuv_ref)))]

    @pl.when(i == 0)
    def _():
        x_copy(0).start()
        cp(0).start()
        cp(1).start()
        x_copy(0).wait()
        cp(0).wait()
        for r in range(1, NR):
            x_copy(r).start()
        cp(2).start()
        for c_ in w_copies():
            c_.start()
        cp(3).start()
        cp(1).wait()
        kb_ref[0:HALO, :] = jnp.zeros((HALO, M), F32)
        vb_ref[0:HALO, :] = jnp.zeros((HALO, M), F32)

    @pl.when(jnp.logical_and(i > 0, i < NR))
    def _():
        x_copy(i).wait()
        kb_ref[0:HALO, :] = kb_ref[RB:RB + HALO, :]
        vb_ref[0:HALO, :] = vb_ref[RB:RB + HALO, :]

    @pl.when(i < NR)
    def _branch_b():
        r0 = pl.multiple_of(i * RB, RB)
        xb = x_ref[pl.ds(r0, RB), :]
        qb = _dot(xb, wqkv_ref[:, 0:M]) * (32 ** -0.5 * LOG2E)
        kb_ref[HALO:, :] = _dot(xb, wqkv_ref[:, M:2 * M])
        vb_ref[HALO:, :] = _dot(xb, wqkv_ref[:, 2 * M:3 * M])
        li = jax.lax.broadcasted_iota(jnp.int32, (128, 128), 0) // 32
        lj = jax.lax.broadcasted_iota(jnp.int32, (128, 128), 1) // 32
        bd = (li == lj).astype(BF16)
        grow = i * RB + jax.lax.broadcasted_iota(jnp.int32, (RB, 128), 0)
        outs = []
        for g in range(M // 128):
            cs = slice(g * 128, (g + 1) * 128)
            qg = qb[:, cs]
            lg = []
            for w in range(8):
                kw = kb_ref[HALO - 2 * w:HALO - 2 * w + RB, cs]
                t = _dot((qg * kw).astype(BF16), bd)
                if w > 0:
                    t = jnp.where(grow >= 2 * w, t, NEG)
                lg.append(t)
            m = functools.reduce(jnp.maximum, lg)
            p = [jnp.exp2(t - m) for t in lg]
            l = functools.reduce(jnp.add, p)
            o = None
            for w in range(8):
                t = p[w] * vb_ref[HALO - 2 * w:HALO - 2 * w + RB, cs]
                o = t if o is None else o + t
            outs.append((o / l).astype(BF16))
        ob = jnp.concatenate(outs, axis=1)
        b = _dot(ob, wob_ref[...])
        gate = jax.nn.sigmoid(jnp.sum(xb.astype(F32) * gw_ref[...].astype(F32), axis=1, keepdims=True))
        g_ref[pl.ds(r0, RB), :] = jnp.broadcast_to(gate, (RB, 128))
        acc_ref[pl.ds(r0, RB), :] = (1.0 - gate) * b

    @pl.when(i == NR)
    def _():
        cp(2).wait()
        for c_ in w_copies():
            c_.wait()

    @pl.when(jnp.logical_and(i >= NR, i < NR + H))
    def _head():
        h = i - NR
        q = (_dot(x_ref[...], _head_weight(wq_ref, h)) * (D ** -0.5 * LOG2E)).astype(BF16)
        k = _dot(c_ref[...], _head_weight(wuk_ref, h)).astype(BF16)
        v = _dot(c_ref[...], _head_weight(wuv_ref, h)).astype(BF16)
        T = 128
        row = jax.lax.broadcasted_iota(jnp.int32, (T, T), 0)
        col = jax.lax.broadcasted_iota(jnp.int32, (T, T), 1)
        tri = col <= row
        for qi in range(S // BQ):
            lo, hi = qi * BQ, (qi + 1) * BQ
            qb = q[lo:hi]
            s1 = _dot_nt(qb, k[:lo + T])
            s2 = jnp.where(tri, _dot_nt(qb[T:], k[lo + T:hi]), NEG)
            s1d = jnp.where(tri, s1[:T, lo:], NEG)
            if qi > 0:
                top = jnp.concatenate([s1[:T, :lo], s1d], axis=1)
            else:
                top = s1d
            bot = s1[T:]
            mt = jnp.max(top, axis=1, keepdims=True)
            mb = jnp.maximum(jnp.max(bot, axis=1, keepdims=True), jnp.max(s2, axis=1, keepdims=True))
            pt = jnp.exp2(top - mt)
            pb = jnp.exp2(bot - mb)
            p2 = jnp.exp2(s2 - mb)
            lt = jnp.sum(pt, axis=1, keepdims=True)
            lb = jnp.sum(pb, axis=1, keepdims=True) + jnp.sum(p2, axis=1, keepdims=True)
            p1 = jnp.concatenate([pt, pb], axis=0).astype(BF16)
            o = _dot(p1, v[:lo + T])
            o2 = _dot(p2.astype(BF16), v[lo + T:hi])
            ctx_ref[h, lo:lo + T, :] = (o[:T] / lt).astype(BF16)
            ctx_ref[h, lo + T:hi, :] = ((o[T:] + o2) / lb).astype(BF16)

    @pl.when(i == NR + H)
    def _():
        cp(3).wait()

    @pl.when(i >= NR + H)
    def _final():
        r0 = pl.multiple_of((i - NR - H) * RB, RB)
        a = _dot(ctx_ref[0, pl.ds(r0, RB), :], wo_ref[0])
        for h in range(1, H):
            a = a + _dot(ctx_ref[h, pl.ds(r0, RB), :], wo_ref[h])
        gate = g_ref[pl.ds(r0, RB), :]
        gate = jnp.concatenate([gate] * (M // 128), axis=1)
        out_ref[...] = (gate * a + acc_ref[pl.ds(r0, RB), :]).astype(out_ref.dtype)


@jax.jit
def pallas_gated_mix__compressed_kv_cla__sliding_local_dilated__prompt_kernel(
        A_x, A_c_kv, A_w_q, A_w_uk, A_w_uv, A_w_o, B_x, B_wqkv, B_wo, gate_w):
    del B_x
    x = A_x.reshape(S, M)
    c = A_c_kv.reshape(S, DC)
    gw = gate_w.reshape(1, M)
    any_spec = pl.BlockSpec(memory_space=pl.ANY)
    out = pl.pallas_call(
        _kernel,
        grid=(NR + H + NR,),
        in_specs=[any_spec] * 8 + [pl.BlockSpec((1, M), lambda i: (0, 0))],
        out_specs=pl.BlockSpec((RB, M), lambda i: (jnp.maximum(i - NR - H, 0), 0)),
        out_shape=jax.ShapeDtypeStruct((S, M), BF16),
        scratch_shapes=[
            pltpu.VMEM((S, M), BF16),
            pltpu.VMEM((S, DC), BF16),
            pltpu.VMEM((H // 2, M, D), U32),
            pltpu.VMEM((H // 2, DC, D), U32),
            pltpu.VMEM((H // 2, DC, D), U32),
            pltpu.VMEM((H, D, M), BF16),
            pltpu.VMEM((M, 3 * M), BF16),
            pltpu.VMEM((M, M), BF16),
            pltpu.VMEM((H, S, D), BF16),
            pltpu.VMEM((S, M), F32),
            pltpu.VMEM((S, 128), F32),
            pltpu.VMEM((HALO + RB, M), F32),
            pltpu.VMEM((HALO + RB, M), F32),
            pltpu.SemaphoreType.DMA((NR,)),
            pltpu.SemaphoreType.DMA((7,)),
        ],
        compiler_params=pltpu.CompilerParams(
            dimension_semantics=("arbitrary",),
            vmem_limit_bytes=120 * 1024 * 1024,
        ),
    )(x, c, A_w_q, A_w_uk, A_w_uv, A_w_o, B_wqkv, B_wo, gw)
    return out.reshape(1, S, M)
```

```python
import jax
import jax.numpy as jnp
import jax.experimental.pallas as pl
import jax.experimental.pallas.tpu as pltpu

S, M, H, D, DC = 2048, 1024, 32, 128, 512
BQ = 256
T = 128
RB = 256
NR = S // RB
HALO = 16
W = 8
NC = M // 128
CH = 16
PCH = 16
LOG2E = 1.4426950408889634
NEG = -1e30
F32, BF16, U32 = jnp.float32, jnp.bfloat16, jnp.uint32
ORDER = (7,6,5,4,3,2,1,0)


def _dot(a, b):
    return jnp.dot(a, b, preferred_element_type=F32)


def _dot_nt(a, b):
    return jax.lax.dot_general(a, b, (((1,), (1,)), ((), ())), preferred_element_type=F32)


def _recip(l):
    r = pl.reciprocal(l, approx=True)
    r = r * (2.0 - l * r)
    return r * (2.0 - l * r)


def _tree(op, xs):
    xs = list(xs)
    while len(xs) > 1:
        xs = [op(xs[j], xs[j + 1]) if j + 1 < len(xs) else xs[j] for j in range(0, len(xs), 2)]
    return xs[0]


def _permute_cols(w_ref, r0):
    lane = jax.lax.broadcasted_iota(jnp.int32, (PCH, 128), 1)
    e, c, hh, f = lane // 64, (lane % 64) // 8, (lane % 8) // 2, lane % 2
    idx = hh * 32 + 4 * c + 2 * e + f
    for m in range(3):
        v = [jnp.take_along_axis(w_ref[pl.ds(r0, PCH), m * M + g * 128:m * M + (g + 1) * 128], idx, axis=1)
             for g in range(NC)]
        for b in (1, 2, 4):
            hi = (c & b) != 0
            nv = list(v)
            for g in range(NC):
                if g & b == 0:
                    nv[g] = jnp.where(hi, pltpu.roll(v[g + b], 8 * b, 1), v[g])
                    nv[g + b] = jnp.where(hi, v[g + b], pltpu.roll(v[g], 128 - 8 * b, 1))
            v = nv
        for g in range(NC):
            w_ref[pl.ds(r0, PCH), m * M + g * 128:m * M + (g + 1) * 128] = v[g]


def _head_weight(w_ref, h):
    w32 = w_ref[h // 2]
    sh = jnp.asarray((1 - h % 2) * 16).astype(U32)
    bits = (w32 << sh) & jnp.uint32(0xFFFF0000)
    return jax.lax.bitcast_convert_type(bits, F32).astype(BF16)


def _kernel(x_hbm, c_hbm, wq_hbm, wuk_hbm, wuv_hbm, wo_hbm, wqkv_hbm, wob_hbm, gw_ref, out_ref,
            x_ref, c_ref, wq_ref, wuk_ref, wuv_ref, wo_ref, wqkv_ref, wob_ref,
            ctx_ref, kb_ref, vb_ref, qs_ref, ps_ref, ob_ref, k_ref, v_ref, sems, wsem):
    i = pl.program_id(0)

    def cp(n):
        wqkv32 = wqkv_hbm.bitcast(U32)
        first, rest = pl.ds(0, 2 * PCH), pl.ds(2 * PCH, M // 2 - 2 * PCH)
        src, dst = ((c_hbm, c_ref), (x_hbm, x_ref), (wo_hbm, wo_ref), (wqkv32.at[rest], wqkv_ref.at[rest]), None,
                    (wqkv32.at[first], wqkv_ref.at[first]))[n]
        return pltpu.make_async_copy(src, dst, sems.at[n])

    def w_copies(j):
        return [pltpu.make_async_copy(src.bitcast(U32).at[:, j, :], dst.at[j], wsem.at[j])
                for src, dst in ((wuk_hbm, wuk_ref), (wuv_hbm, wuv_ref), (wq_hbm, wq_ref))]

    def wob_copies():
        return [pltpu.make_async_copy(wob_hbm.bitcast(U32).at[:, j, :], wob_ref.at[pl.ds(j * 32, 32), :], sems.at[4])
                for j in range(16)]

    def kv_proj(h):
        k_ref[h % 2] = _dot(c_ref[...], _head_weight(wuk_ref, h)).astype(BF16)
        v_ref[h % 2] = _dot(c_ref[...], _head_weight(wuv_ref, h)).astype(BF16)

    @pl.when(i == 0)
    def _():
        cp(0).start()
        for c_ in w_copies(0):
            c_.start()
        cp(1).start()
        cp(5).start()
        cp(0).wait()
        for c_ in w_copies(0):
            c_.wait()
        for c_ in w_copies(1):
            c_.start()
        kv_proj(0)
        cp(1).wait()
        cp(5).wait()
        cp(3).start()

    @pl.when(jnp.logical_and(i < H - 1, i % 2 == 1))
    def _():
        for c_ in w_copies((i + 1) // 2):
            c_.wait()

        @pl.when(i < H - 3)
        def _():
            for c_ in w_copies((i + 1) // 2 + 1):
                c_.start()

    @pl.when(i == 2)
    def _():
        cp(3).wait()

    @pl.when(i == 3)
    def _():
        cp(2).start()

    @pl.when(i == 5)
    def _():
        for c_ in wob_copies():
            c_.start()

    @pl.when(i < H)
    def _head():
        h = i
        _permute_cols(wqkv_ref, pl.multiple_of(h * PCH, PCH))
        wq = _head_weight(wq_ref, h)
        k = k_ref.at[h % 2]
        v = v_ref.at[h % 2]
        row = jax.lax.broadcasted_iota(jnp.int32, (T, T), 0)
        col = jax.lax.broadcasted_iota(jnp.int32, (T, T), 1)
        tri = col <= row
        for qi in ORDER:
            lo, hi = qi * BQ, (qi + 1) * BQ
            qb = (_dot(x_ref[lo:hi, :], wq) * (D ** -0.5 * LOG2E)).astype(BF16)
            s1 = _dot_nt(qb, k[0:lo + T, :])
            s2 = jnp.where(tri, _dot_nt(qb[T:], k[lo + T:hi, :]), NEG)
            s1d = jnp.where(tri, s1[:T, lo:], NEG)
            top = jnp.concatenate([s1[:T, :lo], s1d], axis=1) if qi > 0 else s1d
            bot = s1[T:]
            mt = jnp.max(top, axis=1, keepdims=True)
            mb = jnp.maximum(jnp.max(bot, axis=1, keepdims=True), jnp.max(s2, axis=1, keepdims=True))
            pt = jnp.exp2(top - mt)
            pb = jnp.exp2(bot - mb)
            p2 = jnp.exp2(s2 - mb)
            lt = jnp.sum(pt, axis=1, keepdims=True)
            lb = jnp.sum(pb, axis=1, keepdims=True) + jnp.sum(p2, axis=1, keepdims=True)
            p1 = jnp.concatenate([pt, pb], axis=0).astype(BF16)
            o = _dot(p1, v[0:lo + T, :])
            o2 = _dot(p2.astype(BF16), v[lo + T:hi, :])
            ctx_ref[h, lo:lo + T, :] = (o[:T] * _recip(lt)).astype(BF16)
            ctx_ref[h, lo + T:hi, :] = ((o[T:] + o2) * _recip(lb)).astype(BF16)
        hn = jnp.minimum(h + 1, H - 1)
        k_ref[(h + 1) % 2] = _dot(c_ref[...], _head_weight(wuk_ref, hn)).astype(BF16)
        v_ref[(h + 1) % 2] = _dot(c_ref[...], _head_weight(wuv_ref, hn)).astype(BF16)

    @pl.when(i == H)
    def _():
        kb_ref[:, 0:HALO, :] = jnp.zeros((NC, HALO, 128), F32)
        vb_ref[:, 0:HALO, :] = jnp.zeros((NC, HALO, 128), F32)
        cp(2).wait()
        for c_ in wob_copies():
            c_.wait()

    @pl.when(i > H)
    def _():
        kb_ref[:, 0:HALO, :] = kb_ref[:, RB:RB + HALO, :]
        vb_ref[:, 0:HALO, :] = vb_ref[:, RB:RB + HALO, :]

    @pl.when(i >= H)
    def _last():
        r = i - H
        r0 = pl.multiple_of(r * RB, RB)
        xb = x_ref[pl.ds(r0, RB), :]

        def wcol(n):
            return pltpu.bitcast(wqkv_ref[:, n * 128:(n + 1) * 128], BF16)

        a = [None]

        def a_term(h):
            t = _dot(ctx_ref[h, pl.ds(r0, RB), :], wo_ref[h])
            a[0] = t if a[0] is None else a[0] + t

        for c in range(NC):
            qs_ref[c] = _dot(xb, wcol(c)) * (32 ** -0.5 * LOG2E)
            kb_ref[c, HALO:, :] = _dot(xb, wcol(NC + c))
        even = jax.lax.broadcasted_iota(jnp.int32, (CH, 128), 1) % 2 == 0
        grow = r * RB + jax.lax.broadcasted_iota(jnp.int32, (CH, 128), 0)
        nch = RB // CH
        for ch in range(nch):
            if ch % (nch // NC) == 0:
                c = ch // (nch // NC)
                vb_ref[c, HALO:, :] = _dot(xb, wcol(2 * NC + c))
            a_term(ch)
            lo = ch * CH
            q = [qs_ref[c, lo:lo + CH, :] for c in range(NC)]
            lg = []
            for w in range(W):
                st = HALO - 2 * w + lo
                t = _tree(jnp.add, [q[c] * kb_ref[c, st:st + CH, :] for c in range(NC)])
                t = t + pltpu.roll(t, 64, 1)
                t = t + jnp.where(even, pltpu.roll(t, 127, 1), pltpu.roll(t, 1, 1))
                if w > 0 and lo < HALO:
                    t = jnp.where(grow + lo >= 2 * w, t, NEG)
                lg.append(t)
            m = _tree(jnp.maximum, lg)
            p = [jnp.exp2(t - m) for t in lg]
            rl = _recip(_tree(jnp.add, p))
            for w in range(W):
                ps_ref[w, lo:lo + CH, :] = p[w] * rl
        for ch in range(nch):
            a_term(nch + ch)
            lo = ch * CH
            p = [ps_ref[w, lo:lo + CH, :] for w in range(W)]
            for c in range(NC):
                o = _tree(jnp.add, [p[w] * vb_ref[c, HALO - 2 * w + lo:HALO - 2 * w + lo + CH, :] for w in range(W)])
                ob_ref[lo:lo + CH, c * 128:(c + 1) * 128] = o.astype(BF16)
        b = _dot(ob_ref[...], pltpu.bitcast(wob_ref[...], BF16))
        gate = jax.nn.sigmoid(jnp.sum(xb.astype(F32) * gw_ref[...].astype(F32), axis=1, keepdims=True))
        out_ref[...] = (gate * a[0] + (1.0 - gate) * b).astype(out_ref.dtype)


@jax.jit
def pallas_gated_mix__compressed_kv_cla__sliding_local_dilated__prompt_kernel(
        A_x, A_c_kv, A_w_q, A_w_uk, A_w_uv, A_w_o, B_x, B_wqkv, B_wo, gate_w):
    del B_x
    any_spec = pl.BlockSpec(memory_space=pl.ANY)
    out = pl.pallas_call(
        _kernel,
        grid=(H + NR,),
        in_specs=[any_spec] * 8 + [pl.BlockSpec((1, M), lambda i: (0, 0))],
        out_specs=pl.BlockSpec((RB, M), lambda i: (jnp.maximum(i - H, 0), 0)),
        out_shape=jax.ShapeDtypeStruct((S, M), BF16),
        scratch_shapes=[
            pltpu.VMEM((S, M), BF16),
            pltpu.VMEM((S, DC), BF16),
            pltpu.VMEM((H // 2, M, D), U32),
            pltpu.VMEM((H // 2, DC, D), U32),
            pltpu.VMEM((H // 2, DC, D), U32),
            pltpu.VMEM((H, D, M), BF16),
            pltpu.VMEM((M // 2, 3 * M), U32),
            pltpu.VMEM((M // 2, M), U32),
            pltpu.VMEM((H, S, D), BF16),
            pltpu.VMEM((NC, HALO + RB, 128), F32),
            pltpu.VMEM((NC, HALO + RB, 128), F32),
            pltpu.VMEM((NC, RB, 128), F32),
            pltpu.VMEM((W, RB, 128), F32),
            pltpu.VMEM((RB, M), BF16),
            pltpu.VMEM((2, S, D), BF16),
            pltpu.VMEM((2, S, D), BF16),
            pltpu.SemaphoreType.DMA((6,)),
            pltpu.SemaphoreType.DMA((H // 2,)),
        ],
        compiler_params=pltpu.CompilerParams(
            dimension_semantics=("arbitrary",),
            vmem_limit_bytes=120 * 1024 * 1024,
        ),
    )(A_x.reshape(S, M), A_c_kv.reshape(S, DC), A_w_q, A_w_uk, A_w_uv, A_w_o, B_wqkv,
      B_wo.reshape(32, M // 32, M), gate_w.reshape(1, M))
    return out.reshape(1, S, M)
```

```python
import jax
import jax.numpy as jnp
import jax.experimental.pallas as pl
import jax.experimental.pallas.tpu as pltpu

S, M, H, D, DC = 2048, 1024, 32, 128, 512
BQ = 512
T = 128
RB = 256
NR = S // RB
HALO = 16
W = 8
NC = M // 128
CH = 16
PCH = 16
LOG2E = 1.4426950408889634
NEG = -1e30
F32, BF16, U32 = jnp.float32, jnp.bfloat16, jnp.uint32
ORDER = (3,2,1,0)


def _dot(a, b):
    return jnp.dot(a, b, preferred_element_type=F32)


def _dot_nt(a, b):
    return jax.lax.dot_general(a, b, (((1,), (1,)), ((), ())), preferred_element_type=F32)


def _recip(l):
    r = pl.reciprocal(l, approx=True)
    r = r * (2.0 - l * r)
    return r * (2.0 - l * r)


def _tree(op, xs):
    xs = list(xs)
    while len(xs) > 1:
        xs = [op(xs[j], xs[j + 1]) if j + 1 < len(xs) else xs[j] for j in range(0, len(xs), 2)]
    return xs[0]


def _permute_cols(w_ref, r0):
    lane = jax.lax.broadcasted_iota(jnp.int32, (PCH, 128), 1)
    e, c, hh, f = lane // 64, (lane % 64) // 8, (lane % 8) // 2, lane % 2
    idx = hh * 32 + 4 * c + 2 * e + f
    for m in range(3):
        v = [jnp.take_along_axis(w_ref[pl.ds(r0, PCH), m * M + g * 128:m * M + (g + 1) * 128], idx, axis=1)
             for g in range(NC)]
        for b in (1, 2, 4):
            hi = (c & b) != 0
            nv = list(v)
            for g in range(NC):
                if g & b == 0:
                    nv[g] = jnp.where(hi, pltpu.roll(v[g + b], 8 * b, 1), v[g])
                    nv[g + b] = jnp.where(hi, v[g + b], pltpu.roll(v[g], 128 - 8 * b, 1))
            v = nv
        for g in range(NC):
            w_ref[pl.ds(r0, PCH), m * M + g * 128:m * M + (g + 1) * 128] = v[g]


def _head_weight(w_ref, h):
    w32 = w_ref[h // 2]
    sh = jnp.asarray((1 - h % 2) * 16).astype(U32)
    bits = (w32 << sh) & jnp.uint32(0xFFFF0000)
    return jax.lax.bitcast_convert_type(bits, F32).astype(BF16)


def _kernel(x_hbm, c_hbm, wq_hbm, wuk_hbm, wuv_hbm, wo_hbm, wqkv_hbm, wob_hbm, gw_ref, out_ref,
            x_ref, c_ref, wq_ref, wuk_ref, wuv_ref, wo_ref, wqkv_ref, wob_ref,
            ctx_ref, kb_ref, vb_ref, qs_ref, ps_ref, ob_ref, k_ref, v_ref, sems, wsem):
    i = pl.program_id(0)

    def cp(n):
        wqkv32 = wqkv_hbm.bitcast(U32)
        first, rest = pl.ds(0, 2 * PCH), pl.ds(2 * PCH, M // 2 - 2 * PCH)
        src, dst = ((c_hbm, c_ref), (x_hbm, x_ref), (wo_hbm, wo_ref), (wqkv32.at[rest], wqkv_ref.at[rest]), None,
                    (wqkv32.at[first], wqkv_ref.at[first]))[n]
        return pltpu.make_async_copy(src, dst, sems.at[n])

    def w_copies(j):
        return [pltpu.make_async_copy(src.bitcast(U32).at[:, j, :], dst.at[j], wsem.at[j])
                for src, dst in ((wuk_hbm, wuk_ref), (wuv_hbm, wuv_ref), (wq_hbm, wq_ref))]

    def wob_copies():
        return [pltpu.make_async_copy(wob_hbm.bitcast(U32).at[:, j, :], wob_ref.at[pl.ds(j * 32, 32), :], sems.at[4])
                for j in range(16)]

    def kv_proj(h):
        k_ref[h % 2] = _dot(c_ref[...], _head_weight(wuk_ref, h)).astype(BF16)
        v_ref[h % 2] = _dot(c_ref[...], _head_weight(wuv_ref, h)).astype(BF16)

    @pl.when(i == 0)
    def _():
        cp(0).start()
        for c_ in w_copies(0):
            c_.start()
        cp(1).start()
        cp(5).start()
        cp(0).wait()
        for c_ in w_copies(0):
            c_.wait()
        for c_ in w_copies(1):
            c_.start()
        kv_proj(0)
        cp(1).wait()
        cp(5).wait()
        cp(3).start()

    @pl.when(jnp.logical_and(i < H - 1, i % 2 == 1))
    def _():
        for c_ in w_copies((i + 1) // 2):
            c_.wait()

        @pl.when(i < H - 3)
        def _():
            for c_ in w_copies((i + 1) // 2 + 1):
                c_.start()

    @pl.when(i == 2)
    def _():
        cp(3).wait()

    @pl.when(i == 3)
    def _():
        cp(2).start()

    @pl.when(i == 5)
    def _():
        for c_ in wob_copies():
            c_.start()

    @pl.when(i < H)
    def _head():
        h = i
        _permute_cols(wqkv_ref, pl.multiple_of(h * PCH, PCH))
        wq = _head_weight(wq_ref, h)
        k = k_ref.at[h % 2]
        v = v_ref.at[h % 2]
        row = jax.lax.broadcasted_iota(jnp.int32, (T, T), 0)
        col = jax.lax.broadcasted_iota(jnp.int32, (T, T), 1)
        tri = col <= row
        nb = BQ // T
        for qi in ORDER:
            lo, hi = qi * BQ, (qi + 1) * BQ
            qb = (_dot(x_ref[lo:hi, :], wq) * (D ** -0.5 * LOG2E)).astype(BF16)
            sc = [_dot_nt(qb, k[0:lo + T, :])]
            sc += [_dot_nt(qb[j * T:], k[lo + j * T:lo + (j + 1) * T, :]) for j in range(1, nb)]
            pr, rl = [], []
            for r in range(nb):
                rows = slice(r * T, (r + 1) * T)
                if r == 0:
                    pieces = ([sc[0][rows, :lo]] if lo else []) + [jnp.where(tri, sc[0][rows, lo:], NEG)]
                else:
                    pieces = [sc[0][rows]] + [sc[j][(r - j) * T:(r - j + 1) * T] for j in range(1, r)]
                    pieces.append(jnp.where(tri, sc[r][:T], NEG))
                m = _tree(jnp.maximum, [jnp.max(t, axis=1, keepdims=True) for t in pieces])
                ps = [jnp.exp2(t - m) for t in pieces]
                rl.append(_recip(_tree(jnp.add, [jnp.sum(t, axis=1, keepdims=True) for t in ps])))
                if r == 0 and lo:
                    ps = [jnp.concatenate(ps, axis=1)]
                pr.append([t.astype(BF16) for t in ps])
            o = _dot(jnp.concatenate([pr[r][0] for r in range(nb)], axis=0), v[0:lo + T, :])
            os_ = [o[r * T:(r + 1) * T] for r in range(nb)]
            for j in range(1, nb):
                oj = _dot(jnp.concatenate([pr[r][j] for r in range(j, nb)], axis=0), v[lo + j * T:lo + (j + 1) * T, :])
                for r in range(j, nb):
                    os_[r] = os_[r] + oj[(r - j) * T:(r - j + 1) * T]
            for r in range(nb):
                ctx_ref[h, lo + r * T:lo + (r + 1) * T, :] = (os_[r] * rl[r]).astype(BF16)
        hn = jnp.minimum(h + 1, H - 1)
        k_ref[(h + 1) % 2] = _dot(c_ref[...], _head_weight(wuk_ref, hn)).astype(BF16)
        v_ref[(h + 1) % 2] = _dot(c_ref[...], _head_weight(wuv_ref, hn)).astype(BF16)

    @pl.when(i == H)
    def _():
        kb_ref[:, 0:HALO, :] = jnp.zeros((NC, HALO, 128), F32)
        vb_ref[:, 0:HALO, :] = jnp.zeros((NC, HALO, 128), F32)
        cp(2).wait()
        for c_ in wob_copies():
            c_.wait()

    @pl.when(i > H)
    def _():
        kb_ref[:, 0:HALO, :] = kb_ref[:, RB:RB + HALO, :]
        vb_ref[:, 0:HALO, :] = vb_ref[:, RB:RB + HALO, :]

    @pl.when(i >= H)
    def _last():
        r = i - H
        r0 = pl.multiple_of(r * RB, RB)
        xb = x_ref[pl.ds(r0, RB), :]

        def wcol(n):
            return pltpu.bitcast(wqkv_ref[:, n * 128:(n + 1) * 128], BF16)

        a = [None]

        def a_term(h):
            t = _dot(ctx_ref[h, pl.ds(r0, RB), :], wo_ref[h])
            a[0] = t if a[0] is None else a[0] + t

        for c in range(NC):
            qs_ref[c] = _dot(xb, wcol(c)) * (32 ** -0.5 * LOG2E)
            kb_ref[c, HALO:, :] = _dot(xb, wcol(NC + c))
        even = jax.lax.broadcasted_iota(jnp.int32, (CH, 128), 1) % 2 == 0
        grow = r * RB + jax.lax.broadcasted_iota(jnp.int32, (CH, 128), 0)
        nch = RB // CH
        for ch in range(nch):
            if ch % (nch // NC) == 0:
                c = ch // (nch // NC)
                vb_ref[c, HALO:, :] = _dot(xb, wcol(2 * NC + c))
            a_term(ch)
            lo = ch * CH
            q = [qs_ref[c, lo:lo + CH, :] for c in range(NC)]
            lg = []
            for w in range(W):
                st = HALO - 2 * w + lo
                t = _tree(jnp.add, [q[c] * kb_ref[c, st:st + CH, :] for c in range(NC)])
                t = t + pltpu.roll(t, 64, 1)
                t = t + jnp.where(even, pltpu.roll(t, 127, 1), pltpu.roll(t, 1, 1))
                if w > 0 and lo < HALO:
                    t = jnp.where(grow + lo >= 2 * w, t, NEG)
                lg.append(t)
            m = _tree(jnp.maximum, lg)
            p = [jnp.exp2(t - m) for t in lg]
            rl = _recip(_tree(jnp.add, p))
            for w in range(W):
                ps_ref[w, lo:lo + CH, :] = p[w] * rl
        for ch in range(nch):
            a_term(nch + ch)
            lo = ch * CH
            p = [ps_ref[w, lo:lo + CH, :] for w in range(W)]
            for c in range(NC):
                o = _tree(jnp.add, [p[w] * vb_ref[c, HALO - 2 * w + lo:HALO - 2 * w + lo + CH, :] for w in range(W)])
                ob_ref[lo:lo + CH, c * 128:(c + 1) * 128] = o.astype(BF16)
        b = _dot(ob_ref[...], pltpu.bitcast(wob_ref[...], BF16))
        gate = jax.nn.sigmoid(jnp.sum(xb.astype(F32) * gw_ref[...].astype(F32), axis=1, keepdims=True))
        out_ref[...] = (gate * a[0] + (1.0 - gate) * b).astype(out_ref.dtype)


@jax.jit
def pallas_gated_mix__compressed_kv_cla__sliding_local_dilated__prompt_kernel(
        A_x, A_c_kv, A_w_q, A_w_uk, A_w_uv, A_w_o, B_x, B_wqkv, B_wo, gate_w):
    del B_x
    any_spec = pl.BlockSpec(memory_space=pl.ANY)
    out = pl.pallas_call(
        _kernel,
        grid=(H + NR,),
        in_specs=[any_spec] * 8 + [pl.BlockSpec((1, M), lambda i: (0, 0))],
        out_specs=pl.BlockSpec((RB, M), lambda i: (jnp.maximum(i - H, 0), 0)),
        out_shape=jax.ShapeDtypeStruct((S, M), BF16),
        scratch_shapes=[
            pltpu.VMEM((S, M), BF16),
            pltpu.VMEM((S, DC), BF16),
            pltpu.VMEM((H // 2, M, D), U32),
            pltpu.VMEM((H // 2, DC, D), U32),
            pltpu.VMEM((H // 2, DC, D), U32),
            pltpu.VMEM((H, D, M), BF16),
            pltpu.VMEM((M // 2, 3 * M), U32),
            pltpu.VMEM((M // 2, M), U32),
            pltpu.VMEM((H, S, D), BF16),
            pltpu.VMEM((NC, HALO + RB, 128), F32),
            pltpu.VMEM((NC, HALO + RB, 128), F32),
            pltpu.VMEM((NC, RB, 128), F32),
            pltpu.VMEM((W, RB, 128), F32),
            pltpu.VMEM((RB, M), BF16),
            pltpu.VMEM((2, S, D), BF16),
            pltpu.VMEM((2, S, D), BF16),
            pltpu.SemaphoreType.DMA((6,)),
            pltpu.SemaphoreType.DMA((H // 2,)),
        ],
        compiler_params=pltpu.CompilerParams(
            dimension_semantics=("arbitrary",),
            vmem_limit_bytes=120 * 1024 * 1024,
        ),
    )(A_x.reshape(S, M), A_c_kv.reshape(S, DC), A_w_q, A_w_uk, A_w_uv, A_w_o, B_wqkv,
      B_wo.reshape(32, M // 32, M), gate_w.reshape(1, M))
    return out.reshape(1, S, M)
```

```python
import jax
import jax.numpy as jnp
import jax.experimental.pallas as pl
import jax.experimental.pallas.tpu as pltpu

S, M, H, D, DC = 2048, 1024, 32, 128, 512
BQ = 512
T = 128
RB = 256
NR = S // RB
HALO = 16
W = 8
NC = M // 128
CH = 16
PCH = 16
LOG2E = 1.4426950408889634
NEG = -1e30
F32, BF16, U32 = jnp.float32, jnp.bfloat16, jnp.uint32
ORDER = (3,2,1,0)


def _dot(a, b):
    return jnp.dot(a, b, preferred_element_type=F32)


def _dot_nt(a, b):
    return jax.lax.dot_general(a, b, (((1,), (1,)), ((), ())), preferred_element_type=F32)


def _recip(l):
    r = pl.reciprocal(l, approx=True)
    r = r * (2.0 - l * r)
    return r * (2.0 - l * r)


def _tree(op, xs):
    xs = list(xs)
    while len(xs) > 1:
        xs = [op(xs[j], xs[j + 1]) if j + 1 < len(xs) else xs[j] for j in range(0, len(xs), 2)]
    return xs[0]


def _permute_cols(w_ref, r0):
    lane = jax.lax.broadcasted_iota(jnp.int32, (PCH, 128), 1)
    e, c, hh, f = lane // 64, (lane % 64) // 8, (lane % 8) // 2, lane % 2
    idx = hh * 32 + 4 * c + 2 * e + f
    for m in range(3):
        v = [jnp.take_along_axis(w_ref[pl.ds(r0, PCH), m * M + g * 128:m * M + (g + 1) * 128], idx, axis=1)
             for g in range(NC)]
        for b in (1, 2, 4):
            hi = (c & b) != 0
            nv = list(v)
            for g in range(NC):
                if g & b == 0:
                    nv[g] = jnp.where(hi, pltpu.roll(v[g + b], 8 * b, 1), v[g])
                    nv[g + b] = jnp.where(hi, v[g + b], pltpu.roll(v[g], 128 - 8 * b, 1))
            v = nv
        for g in range(NC):
            w_ref[pl.ds(r0, PCH), m * M + g * 128:m * M + (g + 1) * 128] = v[g]


def _head_weight(w_ref, h):
    w32 = w_ref[h // 2]
    sh = jnp.asarray((1 - h % 2) * 16).astype(U32)
    bits = (w32 << sh) & jnp.uint32(0xFFFF0000)
    return jax.lax.bitcast_convert_type(bits, F32).astype(BF16)


def _kernel(x_hbm, c_hbm, wq_hbm, wuk_hbm, wuv_hbm, wo_hbm, wqkv_hbm, wob_hbm, gw_ref, out_ref,
            x_ref, c_ref, wq_ref, wuk_ref, wuv_ref, wo_ref, wqkv_ref, wob_ref,
            ctx_ref, kb_ref, vb_ref, qs_ref, ps_ref, ob_ref, k_ref, v_ref, sems, wsem):
    i = pl.program_id(0)

    def cp(n):
        wqkv32 = wqkv_hbm.bitcast(U32)
        first, rest = pl.ds(0, 2 * PCH), pl.ds(2 * PCH, M // 2 - 2 * PCH)
        src, dst = ((c_hbm, c_ref), (x_hbm, x_ref), (wo_hbm, wo_ref), (wqkv32.at[rest], wqkv_ref.at[rest]), None,
                    (wqkv32.at[first], wqkv_ref.at[first]))[n]
        return pltpu.make_async_copy(src, dst, sems.at[n])

    def w_copies(j):
        return [pltpu.make_async_copy(src.bitcast(U32).at[:, j, :], dst.at[j], wsem.at[j])
                for src, dst in ((wuk_hbm, wuk_ref), (wuv_hbm, wuv_ref), (wq_hbm, wq_ref))]

    def wob_copies():
        return [pltpu.make_async_copy(wob_hbm.bitcast(U32).at[:, j, :], wob_ref.at[pl.ds(j * 32, 32), :], sems.at[4])
                for j in range(16)]

    def kv_proj(h):
        k_ref[h % 2] = _dot(c_ref[...], _head_weight(wuk_ref, h)).astype(BF16)
        v_ref[h % 2] = _dot(c_ref[...], _head_weight(wuv_ref, h)).astype(BF16)

    @pl.when(i == 0)
    def _():
        cp(0).start()
        for c_ in w_copies(0):
            c_.start()
        cp(1).start()
        cp(5).start()
        cp(0).wait()
        for c_ in w_copies(0):
            c_.wait()
        for c_ in w_copies(1):
            c_.start()
        kv_proj(0)
        cp(1).wait()
        cp(5).wait()
        cp(3).start()

    @pl.when(jnp.logical_and(i < H - 1, i % 2 == 1))
    def _():
        for c_ in w_copies((i + 1) // 2):
            c_.wait()

        @pl.when(i < H - 3)
        def _():
            for c_ in w_copies((i + 1) // 2 + 1):
                c_.start()

    @pl.when(i == 2)
    def _():
        cp(3).wait()

    @pl.when(i == 3)
    def _():
        cp(2).start()

    @pl.when(i == 5)
    def _():
        for c_ in wob_copies():
            c_.start()

    def head_step(last):
        h = i
        _permute_cols(wqkv_ref, pl.multiple_of(h * PCH, PCH))
        wq = _head_weight(wq_ref, h)
        k = k_ref.at[h % 2]
        v = v_ref.at[h % 2]
        row = jax.lax.broadcasted_iota(jnp.int32, (T, T), 0)
        col = jax.lax.broadcasted_iota(jnp.int32, (T, T), 1)
        tri = col <= row
        nb = BQ // T
        for qi in ORDER:
            lo, hi = qi * BQ, (qi + 1) * BQ
            qb = (_dot(x_ref[lo:hi, :], wq) * (D ** -0.5 * LOG2E)).astype(BF16)
            sc = [_dot_nt(qb, k[0:lo + T, :])]
            sc += [_dot_nt(qb[j * T:], k[lo + j * T:lo + (j + 1) * T, :]) for j in range(1, nb)]
            pr, rl = [], []
            for r in range(nb):
                rows = slice(r * T, (r + 1) * T)
                if r == 0:
                    pieces = ([sc[0][rows, :lo]] if lo else []) + [jnp.where(tri, sc[0][rows, lo:], NEG)]
                else:
                    pieces = [sc[0][rows]] + [sc[j][(r - j) * T:(r - j + 1) * T] for j in range(1, r)]
                    pieces.append(jnp.where(tri, sc[r][:T], NEG))
                m = _tree(jnp.maximum, [jnp.max(t, axis=1, keepdims=True) for t in pieces])
                ps = [jnp.exp2(t - m) for t in pieces]
                rl.append(_recip(_tree(jnp.add, [jnp.sum(t, axis=1, keepdims=True) for t in ps])))
                if r == 0 and lo:
                    ps = [jnp.concatenate(ps, axis=1)]
                pr.append([t.astype(BF16) for t in ps])
            o = _dot(jnp.concatenate([pr[r][0] for r in range(nb)], axis=0), v[0:lo + T, :])
            os_ = [o[r * T:(r + 1) * T] for r in range(nb)]
            for j in range(1, nb):
                oj = _dot(jnp.concatenate([pr[r][j] for r in range(j, nb)], axis=0), v[lo + j * T:lo + (j + 1) * T, :])
                for r in range(j, nb):
                    os_[r] = os_[r] + oj[(r - j) * T:(r - j + 1) * T]
            for r in range(nb):
                ctx_ref[h, lo + r * T:lo + (r + 1) * T, :] = (os_[r] * rl[r]).astype(BF16)
        if not last:
            kv_proj(h + 1)

    pl.when(i < H - 1)(lambda: head_step(False))
    pl.when(i == H - 1)(lambda: head_step(True))

    @pl.when(i == H)
    def _():
        kb_ref[:, 0:HALO, :] = jnp.zeros((NC, HALO, 128), F32)
        vb_ref[:, 0:HALO, :] = jnp.zeros((NC, HALO, 128), F32)
        cp(2).wait()
        for c_ in wob_copies():
            c_.wait()

    @pl.when(i > H)
    def _():
        kb_ref[:, 0:HALO, :] = kb_ref[:, RB:RB + HALO, :]
        vb_ref[:, 0:HALO, :] = vb_ref[:, RB:RB + HALO, :]

    @pl.when(i >= H)
    def _last():
        r = i - H
        r0 = pl.multiple_of(r * RB, RB)
        xb = x_ref[pl.ds(r0, RB), :]

        def wcol(n):
            return pltpu.bitcast(wqkv_ref[:, n * 128:(n + 1) * 128], BF16)

        a = [None]

        def a_term(h):
            t = _dot(ctx_ref[h, pl.ds(r0, RB), :], wo_ref[h])
            a[0] = t if a[0] is None else a[0] + t

        for c in range(NC):
            qs_ref[c] = _dot(xb, wcol(c)) * (32 ** -0.5 * LOG2E)
            kb_ref[c, HALO:, :] = _dot(xb, wcol(NC + c))
        even = jax.lax.broadcasted_iota(jnp.int32, (CH, 128), 1) % 2 == 0
        grow = r * RB + jax.lax.broadcasted_iota(jnp.int32, (CH, 128), 0)
        nch = RB // CH
        for ch in range(nch):
            if ch % (nch // NC) == 0:
                c = ch // (nch // NC)
                vb_ref[c, HALO:, :] = _dot(xb, wcol(2 * NC + c))
            a_term(ch)
            lo = ch * CH
            q = [qs_ref[c, lo:lo + CH, :] for c in range(NC)]
            lg = []
            for w in range(W):
                st = HALO - 2 * w + lo
                t = _tree(jnp.add, [q[c] * kb_ref[c, st:st + CH, :] for c in range(NC)])
                t = t + pltpu.roll(t, 64, 1)
                t = t + jnp.where(even, pltpu.roll(t, 127, 1), pltpu.roll(t, 1, 1))
                if w > 0 and lo < HALO:
                    t = jnp.where(grow + lo >= 2 * w, t, NEG)
                lg.append(t)
            m = _tree(jnp.maximum, lg)
            p = [jnp.exp2(t - m) for t in lg]
            rl = _recip(_tree(jnp.add, p))
            for w in range(W):
                ps_ref[w, lo:lo + CH, :] = p[w] * rl
        for ch in range(nch):
            a_term(nch + ch)
            lo = ch * CH
            p = [ps_ref[w, lo:lo + CH, :] for w in range(W)]
            for c in range(NC):
                o = _tree(jnp.add, [p[w] * vb_ref[c, HALO - 2 * w + lo:HALO - 2 * w + lo + CH, :] for w in range(W)])
                ob_ref[lo:lo + CH, c * 128:(c + 1) * 128] = o.astype(BF16)
        b = _dot(ob_ref[...], pltpu.bitcast(wob_ref[...], BF16))
        gate = jax.nn.sigmoid(jnp.sum(xb.astype(F32) * gw_ref[...].astype(F32), axis=1, keepdims=True))
        out_ref[...] = (gate * a[0] + (1.0 - gate) * b).astype(out_ref.dtype)


@jax.jit
def pallas_gated_mix__compressed_kv_cla__sliding_local_dilated__prompt_kernel(
        A_x, A_c_kv, A_w_q, A_w_uk, A_w_uv, A_w_o, B_x, B_wqkv, B_wo, gate_w):
    del B_x
    any_spec = pl.BlockSpec(memory_space=pl.ANY)
    out = pl.pallas_call(
        _kernel,
        grid=(H + NR,),
        in_specs=[any_spec] * 8 + [pl.BlockSpec((1, M), lambda i: (0, 0))],
        out_specs=pl.BlockSpec((RB, M), lambda i: (jnp.maximum(i - H, 0), 0)),
        out_shape=jax.ShapeDtypeStruct((S, M), BF16),
        scratch_shapes=[
            pltpu.VMEM((S, M), BF16),
            pltpu.VMEM((S, DC), BF16),
            pltpu.VMEM((H // 2, M, D), U32),
            pltpu.VMEM((H // 2, DC, D), U32),
            pltpu.VMEM((H // 2, DC, D), U32),
            pltpu.VMEM((H, D, M), BF16),
            pltpu.VMEM((M // 2, 3 * M), U32),
            pltpu.VMEM((M // 2, M), U32),
            pltpu.VMEM((H, S, D), BF16),
            pltpu.VMEM((NC, HALO + RB, 128), F32),
            pltpu.VMEM((NC, HALO + RB, 128), F32),
            pltpu.VMEM((NC, RB, 128), F32),
            pltpu.VMEM((W, RB, 128), F32),
            pltpu.VMEM((RB, M), BF16),
            pltpu.VMEM((2, S, D), BF16),
            pltpu.VMEM((2, S, D), BF16),
            pltpu.SemaphoreType.DMA((6,)),
            pltpu.SemaphoreType.DMA((H // 2,)),
        ],
        compiler_params=pltpu.CompilerParams(
            dimension_semantics=("arbitrary",),
            vmem_limit_bytes=120 * 1024 * 1024,
        ),
    )(A_x.reshape(S, M), A_c_kv.reshape(S, DC), A_w_q, A_w_uk, A_w_uv, A_w_o, B_wqkv,
      B_wo.reshape(32, M // 32, M), gate_w.reshape(1, M))
    return out.reshape(1, S, M)
```

```python
import jax
import jax.numpy as jnp
import jax.experimental.pallas as pl
import jax.experimental.pallas.tpu as pltpu

S, M, H, D, DC = 2048, 1024, 32, 128, 512
BQ = 512
T = 128
RB = 256
NR = S // RB
HALO = 16
W = 8
NC = M // 128
CH = 16
PCH = 16
LOG2E = 1.4426950408889634
NEG = -1e30
F32, BF16, U32 = jnp.float32, jnp.bfloat16, jnp.uint32
ORDER = (3,2,1,0)


def _dot(a, b):
    return jnp.dot(a, b, preferred_element_type=F32)


def _dot_nt(a, b):
    return jax.lax.dot_general(a, b, (((1,), (1,)), ((), ())), preferred_element_type=F32)


def _recip(l):
    r = pl.reciprocal(l, approx=True)
    r = r * (2.0 - l * r)
    return r * (2.0 - l * r)


def _tree(op, xs):
    xs = list(xs)
    while len(xs) > 1:
        xs = [op(xs[j], xs[j + 1]) if j + 1 < len(xs) else xs[j] for j in range(0, len(xs), 2)]
    return xs[0]


def _permute_cols(w_ref, r0):
    lane = jax.lax.broadcasted_iota(jnp.int32, (PCH, 128), 1)
    e, c, hh, f = lane // 64, (lane % 64) // 8, (lane % 8) // 2, lane % 2
    idx = hh * 32 + 4 * c + 2 * e + f
    for m in range(3):
        v = [jnp.take_along_axis(w_ref[pl.ds(r0, PCH), m * M + g * 128:m * M + (g + 1) * 128], idx, axis=1)
             for g in range(NC)]
        for b in (1, 2, 4):
            hi = (c & b) != 0
            nv = list(v)
            for g in range(NC):
                if g & b == 0:
                    nv[g] = jnp.where(hi, pltpu.roll(v[g + b], 8 * b, 1), v[g])
                    nv[g + b] = jnp.where(hi, v[g + b], pltpu.roll(v[g], 128 - 8 * b, 1))
            v = nv
        for g in range(NC):
            w_ref[pl.ds(r0, PCH), m * M + g * 128:m * M + (g + 1) * 128] = v[g]


def _head_weight(w_ref, h):
    w32 = w_ref[h // 2]
    sh = jnp.asarray((1 - h % 2) * 16, jnp.int32).astype(U32)
    bits = (w32 << sh) & jnp.uint32(0xFFFF0000)
    return jax.lax.bitcast_convert_type(bits, F32).astype(BF16)


def _kernel(x_hbm, c_hbm, wq_hbm, wuk_hbm, wuv_hbm, wo_hbm, wqkv_hbm, wob_hbm, gw_ref, out_ref,
            x_ref, c_ref, wq_ref, wuk_ref, wuv_ref, wo_ref, wqkv_ref, wob_ref,
            ctx_ref, kb_ref, vb_ref, qs_ref, ps_ref, ob_ref, k_ref, v_ref, sems, wsem):
    step = pl.program_id(0)

    def cp(n):
        wqkv32 = wqkv_hbm.bitcast(U32)
        first, rest = pl.ds(0, 2 * PCH), pl.ds(2 * PCH, M // 2 - 2 * PCH)
        src, dst = ((c_hbm, c_ref), (x_hbm, x_ref), (wo_hbm, wo_ref), (wqkv32.at[rest], wqkv_ref.at[rest]), None,
                    (wqkv32.at[first], wqkv_ref.at[first]))[n]
        return pltpu.make_async_copy(src, dst, sems.at[n])

    def w_copies(j):
        return [pltpu.make_async_copy(src.bitcast(U32).at[:, j, :], dst.at[j], wsem.at[j])
                for src, dst in ((wuk_hbm, wuk_ref), (wuv_hbm, wuv_ref), (wq_hbm, wq_ref))]

    def wob_copies():
        return [pltpu.make_async_copy(wob_hbm.bitcast(U32).at[:, j, :], wob_ref.at[pl.ds(j * 32, 32), :], sems.at[4])
                for j in range(16)]

    def kv_proj(h):
        k_ref[h % 2] = _dot(c_ref[...], _head_weight(wuk_ref, h)).astype(BF16)
        v_ref[h % 2] = _dot(c_ref[...], _head_weight(wuv_ref, h)).astype(BF16)

    @pl.when(step == 0)
    def _():
        cp(0).start()
        for c_ in w_copies(0):
            c_.start()
        cp(1).start()
        cp(5).start()
        cp(0).wait()
        for c_ in w_copies(0):
            c_.wait()
        for c_ in w_copies(1):
            c_.start()
        kv_proj(0)
        cp(1).wait()
        cp(5).wait()
        cp(3).start()

    def head_step(h, last):
        _permute_cols(wqkv_ref, pl.multiple_of(h * PCH, PCH))
        wq = _head_weight(wq_ref, h)
        k = k_ref.at[h % 2]
        v = v_ref.at[h % 2]
        row = jax.lax.broadcasted_iota(jnp.int32, (T, T), 0)
        col = jax.lax.broadcasted_iota(jnp.int32, (T, T), 1)
        tri = col <= row
        nb = BQ // T
        for qi in ORDER:
            lo, hi = qi * BQ, (qi + 1) * BQ
            qb = (_dot(x_ref[lo:hi, :], wq) * (D ** -0.5 * LOG2E)).astype(BF16)
            sc = [_dot_nt(qb, k[0:lo + T, :])]
            sc += [_dot_nt(qb[j * T:], k[lo + j * T:lo + (j + 1) * T, :]) for j in range(1, nb)]
            pr, rl = [], []
            for r in range(nb):
                rows = slice(r * T, (r + 1) * T)
                if r == 0:
                    pieces = ([sc[0][rows, :lo]] if lo else []) + [jnp.where(tri, sc[0][rows, lo:], NEG)]
                else:
                    pieces = [sc[0][rows]] + [sc[j][(r - j) * T:(r - j + 1) * T] for j in range(1, r)]
                    pieces.append(jnp.where(tri, sc[r][:T], NEG))
                m = _tree(jnp.maximum, [jnp.max(t, axis=1, keepdims=True) for t in pieces])
                ps = [jnp.exp2(t - m) for t in pieces]
                rl.append(_recip(_tree(jnp.add, [jnp.sum(t, axis=1, keepdims=True) for t in ps])))
                if r == 0 and lo:
                    ps = [jnp.concatenate(ps, axis=1)]
                pr.append([t.astype(BF16) for t in ps])
            o = _dot(jnp.concatenate([pr[r][0] for r in range(nb)], axis=0), v[0:lo + T, :])
            os_ = [o[r * T:(r + 1) * T] for r in range(nb)]
            for j in range(1, nb):
                oj = _dot(jnp.concatenate([pr[r][j] for r in range(j, nb)], axis=0), v[lo + j * T:lo + (j + 1) * T, :])
                for r in range(j, nb):
                    os_[r] = os_[r] + oj[(r - j) * T:(r - j + 1) * T]
            for r in range(nb):
                ctx_ref[h, lo + r * T:lo + (r + 1) * T, :] = (os_[r] * rl[r]).astype(BF16)
        if not last:
            kv_proj(h + 1)

    @pl.when(step == 0)
    def _():
        @pl.loop(0, H - 1)
        def _(i):
            @pl.when(jnp.logical_and(i < H - 1, i % 2 == 1))
            def _():
                for c_ in w_copies((i + 1) // 2):
                    c_.wait()

                @pl.when(i < H - 3)
                def _():
                    for c_ in w_copies((i + 1) // 2 + 1):
                        c_.start()

            @pl.when(i == 2)
            def _():
                cp(3).wait()

            @pl.when(i == 3)
            def _():
                cp(2).start()

            @pl.when(i == 5)
            def _():
                for c_ in wob_copies():
                    c_.start()

            head_step(i, False)

        head_step(H - 1, True)

    i = step + (H - 1)
    @pl.when(i == H)
    def _():
        kb_ref[:, 0:HALO, :] = jnp.zeros((NC, HALO, 128), F32)
        vb_ref[:, 0:HALO, :] = jnp.zeros((NC, HALO, 128), F32)
        cp(2).wait()
        for c_ in wob_copies():
            c_.wait()

    @pl.when(i > H)
    def _():
        kb_ref[:, 0:HALO, :] = kb_ref[:, RB:RB + HALO, :]
        vb_ref[:, 0:HALO, :] = vb_ref[:, RB:RB + HALO, :]

    @pl.when(i >= H)
    def _last():
        r = i - H
        r0 = pl.multiple_of(r * RB, RB)
        xb = x_ref[pl.ds(r0, RB), :]

        def wcol(n):
            return pltpu.bitcast(wqkv_ref[:, n * 128:(n + 1) * 128], BF16)

        a = [None]

        def a_term(h):
            t = _dot(ctx_ref[h, pl.ds(r0, RB), :], wo_ref[h])
            a[0] = t if a[0] is None else a[0] + t

        for c in range(NC):
            qs_ref[c] = _dot(xb, wcol(c)) * (32 ** -0.5 * LOG2E)
            kb_ref[c, HALO:, :] = _dot(xb, wcol(NC + c))
        even = jax.lax.broadcasted_iota(jnp.int32, (CH, 128), 1) % 2 == 0
        grow = r * RB + jax.lax.broadcasted_iota(jnp.int32, (CH, 128), 0)
        nch = RB // CH
        for ch in range(nch):
            if ch % (nch // NC) == 0:
                c = ch // (nch // NC)
                vb_ref[c, HALO:, :] = _dot(xb, wcol(2 * NC + c))
            a_term(ch)
            lo = ch * CH
            q = [qs_ref[c, lo:lo + CH, :] for c in range(NC)]
            lg = []
            for w in range(W):
                st = HALO - 2 * w + lo
                t = _tree(jnp.add, [q[c] * kb_ref[c, st:st + CH, :] for c in range(NC)])
                t = t + pltpu.roll(t, 64, 1)
                t = t + jnp.where(even, pltpu.roll(t, 127, 1), pltpu.roll(t, 1, 1))
                if w > 0 and lo < HALO:
                    t = jnp.where(grow + lo >= 2 * w, t, NEG)
                lg.append(t)
            m = _tree(jnp.maximum, lg)
            p = [jnp.exp2(t - m) for t in lg]
            rl = _recip(_tree(jnp.add, p))
            for w in range(W):
                ps_ref[w, lo:lo + CH, :] = p[w] * rl
        for ch in range(nch):
            a_term(nch + ch)
            lo = ch * CH
            p = [ps_ref[w, lo:lo + CH, :] for w in range(W)]
            for c in range(NC):
                o = _tree(jnp.add, [p[w] * vb_ref[c, HALO - 2 * w + lo:HALO - 2 * w + lo + CH, :] for w in range(W)])
                ob_ref[lo:lo + CH, c * 128:(c + 1) * 128] = o.astype(BF16)
        b = _dot(ob_ref[...], pltpu.bitcast(wob_ref[...], BF16))
        gate = jax.nn.sigmoid(jnp.sum(xb.astype(F32) * gw_ref[...].astype(F32), axis=1, keepdims=True))
        out_ref[...] = (gate * a[0] + (1.0 - gate) * b).astype(out_ref.dtype)


@jax.jit
def pallas_gated_mix__compressed_kv_cla__sliding_local_dilated__prompt_kernel(
        A_x, A_c_kv, A_w_q, A_w_uk, A_w_uv, A_w_o, B_x, B_wqkv, B_wo, gate_w):
    del B_x
    any_spec = pl.BlockSpec(memory_space=pl.ANY)
    out = pl.pallas_call(
        _kernel,
        grid=(1 + NR,),
        in_specs=[any_spec] * 8 + [pl.BlockSpec((1, M), lambda i: (0, 0))],
        out_specs=pl.BlockSpec((RB, M), lambda i: (jnp.maximum(i - 1, 0), 0)),
        out_shape=jax.ShapeDtypeStruct((S, M), BF16),
        scratch_shapes=[
            pltpu.VMEM((S, M), BF16),
            pltpu.VMEM((S, DC), BF16),
            pltpu.VMEM((H // 2, M, D), U32),
            pltpu.VMEM((H // 2, DC, D), U32),
            pltpu.VMEM((H // 2, DC, D), U32),
            pltpu.VMEM((H, D, M), BF16),
            pltpu.VMEM((M // 2, 3 * M), U32),
            pltpu.VMEM((M // 2, M), U32),
            pltpu.VMEM((H, S, D), BF16),
            pltpu.VMEM((NC, HALO + RB, 128), F32),
            pltpu.VMEM((NC, HALO + RB, 128), F32),
            pltpu.VMEM((NC, RB, 128), F32),
            pltpu.VMEM((W, RB, 128), F32),
            pltpu.VMEM((RB, M), BF16),
            pltpu.VMEM((2, S, D), BF16),
            pltpu.VMEM((2, S, D), BF16),
            pltpu.SemaphoreType.DMA((6,)),
            pltpu.SemaphoreType.DMA((H // 2,)),
        ],
        compiler_params=pltpu.CompilerParams(
            dimension_semantics=("arbitrary",),
            vmem_limit_bytes=120 * 1024 * 1024,
        ),
    )(A_x.reshape(S, M), A_c_kv.reshape(S, DC), A_w_q, A_w_uk, A_w_uv, A_w_o, B_wqkv,
      B_wo.reshape(32, M // 32, M), gate_w.reshape(1, M))
    return out.reshape(1, S, M)
```

```python
import jax
import jax.numpy as jnp
import jax.experimental.pallas as pl
import jax.experimental.pallas.tpu as pltpu

S, M, H, D, DC = 2048, 1024, 32, 128, 512
BQ = 512
T = 128
RB = 256
NR = S // RB
HALO = 16
W = 8
NC = M // 128
CH = 16
PCH = 16
LOG2E = 1.4426950408889634
NEG = -1e30
F32, BF16, U32 = jnp.float32, jnp.bfloat16, jnp.uint32
ORDER = (3,1,2,0)
ORDER_LAST = (3, 0, 2, 1)


def _dot(a, b):
    return jnp.dot(a, b, preferred_element_type=F32)


def _dot_nt(a, b):
    return jax.lax.dot_general(a, b, (((1,), (1,)), ((), ())), preferred_element_type=F32)


def _recip(l):
    r = pl.reciprocal(l, approx=True)
    r = r * (2.0 - l * r)
    return r * (2.0 - l * r)


def _tree(op, xs):
    xs = list(xs)
    while len(xs) > 1:
        xs = [op(xs[j], xs[j + 1]) if j + 1 < len(xs) else xs[j] for j in range(0, len(xs), 2)]
    return xs[0]


def _permute_cols(w_ref, r0):
    lane = jax.lax.broadcasted_iota(jnp.int32, (PCH, 128), 1)
    e, c, hh, f = lane // 64, (lane % 64) // 8, (lane % 8) // 2, lane % 2
    idx = hh * 32 + 4 * c + 2 * e + f
    for m in range(3):
        v = [jnp.take_along_axis(w_ref[pl.ds(r0, PCH), m * M + g * 128:m * M + (g + 1) * 128], idx, axis=1)
             for g in range(NC)]
        for b in (1, 2, 4):
            hi = (c & b) != 0
            nv = list(v)
            for g in range(NC):
                if g & b == 0:
                    nv[g] = jnp.where(hi, pltpu.roll(v[g + b], 8 * b, 1), v[g])
                    nv[g + b] = jnp.where(hi, v[g + b], pltpu.roll(v[g], 128 - 8 * b, 1))
            v = nv
        for g in range(NC):
            w_ref[pl.ds(r0, PCH), m * M + g * 128:m * M + (g + 1) * 128] = v[g]


def _head_weight(w_ref, h):
    w32 = w_ref[h // 2]
    sh = jnp.asarray((1 - h % 2) * 16, jnp.int32).astype(U32)
    bits = (w32 << sh) & jnp.uint32(0xFFFF0000)
    return jax.lax.bitcast_convert_type(bits, F32).astype(BF16)


def _kernel(x_hbm, c_hbm, wq_hbm, wuk_hbm, wuv_hbm, wo_hbm, wqkv_hbm, wob_hbm, gw_ref, out_hbm,
            x_ref, c_ref, wq_ref, wuk_ref, wuv_ref, wo_ref, wqkv_ref, wob_ref,
            ctx_ref, kb_ref, vb_ref, qs_ref, ps_ref, ob_ref, k_ref, v_ref, o_ref, sems, wsem, osem):

    def cp(n):
        wqkv32 = wqkv_hbm.bitcast(U32)
        first, rest = pl.ds(0, 2 * PCH), pl.ds(2 * PCH, M // 2 - 2 * PCH)
        src, dst = ((c_hbm, c_ref), (x_hbm, x_ref), (wo_hbm, wo_ref), (wqkv32.at[rest], wqkv_ref.at[rest]), None,
                    (wqkv32.at[first], wqkv_ref.at[first]))[n]
        return pltpu.make_async_copy(src, dst, sems.at[n])

    def w_copies(j):
        return [pltpu.make_async_copy(src.bitcast(U32).at[:, j, :], dst.at[j], wsem.at[j])
                for src, dst in ((wuk_hbm, wuk_ref), (wuv_hbm, wuv_ref), (wq_hbm, wq_ref))]

    def wob_copies():
        return [pltpu.make_async_copy(wob_hbm.bitcast(U32).at[:, j, :], wob_ref.at[pl.ds(j * 32, 32), :], sems.at[4])
                for j in range(16)]

    def kv_proj(h):
        k_ref[h % 2] = _dot(c_ref[...], _head_weight(wuk_ref, h)).astype(BF16)
        v_ref[h % 2] = _dot(c_ref[...], _head_weight(wuv_ref, h)).astype(BF16)

    def prologue():
        cp(0).start()
        for c_ in w_copies(0):
            c_.start()
        cp(1).start()
        cp(5).start()
        cp(0).wait()
        for c_ in w_copies(0):
            c_.wait()
        for c_ in w_copies(1):
            c_.start()
        kv_proj(0)
        cp(1).wait()
        cp(5).wait()
        cp(3).start()

    def head_step(h, last):
        _permute_cols(wqkv_ref, pl.multiple_of(h * PCH, PCH))
        wq = _head_weight(wq_ref, h)
        k = k_ref.at[h % 2]
        v = v_ref.at[h % 2]
        row = jax.lax.broadcasted_iota(jnp.int32, (T, T), 0)
        col = jax.lax.broadcasted_iota(jnp.int32, (T, T), 1)
        tri = col <= row
        nb = BQ // T
        for qi in (ORDER_LAST if last else ORDER):
            lo, hi = qi * BQ, (qi + 1) * BQ
            qb = (_dot(x_ref[lo:hi, :], wq) * (D ** -0.5 * LOG2E)).astype(BF16)
            sc = [_dot_nt(qb, k[0:lo + T, :])]
            sc += [_dot_nt(qb[j * T:], k[lo + j * T:lo + (j + 1) * T, :]) for j in range(1, nb)]
            pr, rl = [], []
            for r in range(nb):
                rows = slice(r * T, (r + 1) * T)
                if r == 0:
                    pieces = ([sc[0][rows, :lo]] if lo else []) + [jnp.where(tri, sc[0][rows, lo:], NEG)]
                else:
                    pieces = [sc[0][rows]] + [sc[j][(r - j) * T:(r - j + 1) * T] for j in range(1, r)]
                    pieces.append(jnp.where(tri, sc[r][:T], NEG))
                m = _tree(jnp.maximum, [jnp.max(t, axis=1, keepdims=True) for t in pieces])
                ps = [jnp.exp2(t - m) for t in pieces]
                rl.append(_recip(_tree(jnp.add, [jnp.sum(t, axis=1, keepdims=True) for t in ps])))
                if r == 0 and lo:
                    ps = [jnp.concatenate(ps, axis=1)]
                pr.append([t.astype(BF16) for t in ps])
            o = _dot(jnp.concatenate([pr[r][0] for r in range(nb)], axis=0), v[0:lo + T, :])
            os_ = [o[r * T:(r + 1) * T] for r in range(nb)]
            for j in range(1, nb):
                oj = _dot(jnp.concatenate([pr[r][j] for r in range(j, nb)], axis=0), v[lo + j * T:lo + (j + 1) * T, :])
                for r in range(j, nb):
                    os_[r] = os_[r] + oj[(r - j) * T:(r - j + 1) * T]
            for r in range(nb):
                ctx_ref[h, lo + r * T:lo + (r + 1) * T, :] = (os_[r] * rl[r]).astype(BF16)
        if not last:
            kv_proj(h + 1)

    prologue()

    @pl.loop(0, H - 1)
    def _(i):
        head_step(i, False)

        @pl.when(jnp.logical_and(i < H - 2, i % 2 == 0))
        def _():
            for c_ in w_copies(i // 2 + 1):
                c_.wait()

            @pl.when(i < H - 4)
            def _():
                for c_ in w_copies(i // 2 + 2):
                    c_.start()

        @pl.when(i == 1)
        def _():
            cp(3).wait()

        @pl.when(i == 2)
        def _():
            cp(2).start()

        @pl.when(i == 4)
        def _():
            for c_ in wob_copies():
                c_.start()


    head_step(H - 1, True)

    kb_ref[:, RB:RB + HALO, :] = jnp.zeros((NC, HALO, 128), F32)
    vb_ref[:, RB:RB + HALO, :] = jnp.zeros((NC, HALO, 128), F32)
    cp(2).wait()
    for c_ in wob_copies():
        c_.wait()

    def out_copy(r):
        return pltpu.make_async_copy(o_ref.at[r % 2], out_hbm.at[pl.ds(r * RB, RB), :], osem.at[r % 2])

    @pl.loop(0, NR)
    def _(r):
        @pl.when(r >= 2)
        def _():
            out_copy(r - 2).wait()
        kb_ref[:, 0:HALO, :] = kb_ref[:, RB:RB + HALO, :]
        vb_ref[:, 0:HALO, :] = vb_ref[:, RB:RB + HALO, :]
        r0 = pl.multiple_of(r * RB, RB)
        xb = x_ref[pl.ds(r0, RB), :]

        def wcol(n):
            return pltpu.bitcast(wqkv_ref[:, n * 128:(n + 1) * 128], BF16)

        a = [None]

        def a_term(h):
            t = _dot(ctx_ref[h, pl.ds(r0, RB), :], wo_ref[h])
            a[0] = t if a[0] is None else a[0] + t

        for c in range(NC):
            qs_ref[c] = _dot(xb, wcol(c)) * (32 ** -0.5 * LOG2E)
            kb_ref[c, HALO:, :] = _dot(xb, wcol(NC + c))
        even = jax.lax.broadcasted_iota(jnp.int32, (CH, 128), 1) % 2 == 0
        grow = r * RB + jax.lax.broadcasted_iota(jnp.int32, (CH, 128), 0)
        nch = RB // CH
        for ch in range(nch):
            if ch % (nch // NC) == 0:
                c = ch // (nch // NC)
                vb_ref[c, HALO:, :] = _dot(xb, wcol(2 * NC + c))
            a_term(ch)
            lo = ch * CH
            q = [qs_ref[c, lo:lo + CH, :] for c in range(NC)]
            lg = []
            for w in range(W):
                st = HALO - 2 * w + lo
                t = _tree(jnp.add, [q[c] * kb_ref[c, st:st + CH, :] for c in range(NC)])
                t = t + pltpu.roll(t, 64, 1)
                t = t + jnp.where(even, pltpu.roll(t, 127, 1), pltpu.roll(t, 1, 1))
                if w > 0 and lo < HALO:
                    t = jnp.where(grow + lo >= 2 * w, t, NEG)
                lg.append(t)
            m = _tree(jnp.maximum, lg)
            p = [jnp.exp2(t - m) for t in lg]
            rl = _recip(_tree(jnp.add, p))
            for w in range(W):
                ps_ref[w, lo:lo + CH, :] = p[w] * rl
        for ch in range(nch):
            a_term(nch + ch)
            lo = ch * CH
            p = [ps_ref[w, lo:lo + CH, :] for w in range(W)]
            for c in range(NC):
                o = _tree(jnp.add, [p[w] * vb_ref[c, HALO - 2 * w + lo:HALO - 2 * w + lo + CH, :] for w in range(W)])
                ob_ref[lo:lo + CH, c * 128:(c + 1) * 128] = o.astype(BF16)
        b = _dot(ob_ref[...], pltpu.bitcast(wob_ref[...], BF16))
        gate = jax.nn.sigmoid(jnp.sum(xb.astype(F32) * gw_ref[...].astype(F32), axis=1, keepdims=True))
        o_ref[r % 2] = (gate * a[0] + (1.0 - gate) * b).astype(o_ref.dtype)
        out_copy(r).start()

    out_copy(NR - 2).wait()
    out_copy(NR - 1).wait()


@jax.jit
def pallas_gated_mix__compressed_kv_cla__sliding_local_dilated__prompt_kernel(
        A_x, A_c_kv, A_w_q, A_w_uk, A_w_uv, A_w_o, B_x, B_wqkv, B_wo, gate_w):
    del B_x
    any_spec = pl.BlockSpec(memory_space=pl.ANY)
    out = pl.pallas_call(
        _kernel,
        in_specs=[any_spec] * 8 + [pl.BlockSpec(memory_space=pltpu.VMEM)],
        out_specs=any_spec,
        out_shape=jax.ShapeDtypeStruct((S, M), BF16),
        scratch_shapes=[
            pltpu.VMEM((S, M), BF16),
            pltpu.VMEM((S, DC), BF16),
            pltpu.VMEM((H // 2, M, D), U32),
            pltpu.VMEM((H // 2, DC, D), U32),
            pltpu.VMEM((H // 2, DC, D), U32),
            pltpu.VMEM((H, D, M), BF16),
            pltpu.VMEM((M // 2, 3 * M), U32),
            pltpu.VMEM((M // 2, M), U32),
            pltpu.VMEM((H, S, D), BF16),
            pltpu.VMEM((NC, HALO + RB, 128), F32),
            pltpu.VMEM((NC, HALO + RB, 128), F32),
            pltpu.VMEM((NC, RB, 128), F32),
            pltpu.VMEM((W, RB, 128), F32),
            pltpu.VMEM((RB, M), BF16),
            pltpu.VMEM((2, S, D), BF16),
            pltpu.VMEM((2, S, D), BF16),
            pltpu.VMEM((2, RB, M), BF16),
            pltpu.SemaphoreType.DMA((6,)),
            pltpu.SemaphoreType.DMA((H // 2,)),
            pltpu.SemaphoreType.DMA((2,)),
        ],
        compiler_params=pltpu.CompilerParams(
            vmem_limit_bytes=120 * 1024 * 1024,
        ),
    )(A_x.reshape(S, M), A_c_kv.reshape(S, DC), A_w_q, A_w_uk, A_w_uv, A_w_o, B_wqkv,
      B_wo.reshape(32, M // 32, M), gate_w.reshape(1, M))
    return out.reshape(1, S, M)
```

```python
import jax
import jax.numpy as jnp
import jax.experimental.pallas as pl
import jax.experimental.pallas.tpu as pltpu

S, M, H, D, DC = 2048, 1024, 32, 128, 512
BQ = 512
T = 128
RB = 256
NR = S // RB
HALO = 16
W = 8
NC = M // 128
CH = 16
PCH = 16
LOG2E = 1.4426950408889634
NEG = -1e30
F32, BF16, U32 = jnp.float32, jnp.bfloat16, jnp.uint32
ORDER = (3, 1, 2, 0)
ORDER_LAST = (3, 0, 2, 1)


def _dot(a, b):
    return jnp.dot(a, b, preferred_element_type=F32)


def _dot_nt(a, b):
    return jax.lax.dot_general(a, b, (((1,), (1,)), ((), ())), preferred_element_type=F32)


def _recip(l):
    r = pl.reciprocal(l, approx=True)
    r = r * (2.0 - l * r)
    return r * (2.0 - l * r)


def _tree(op, xs):
    xs = list(xs)
    while len(xs) > 1:
        xs = [op(xs[j], xs[j + 1]) if j + 1 < len(xs) else xs[j] for j in range(0, len(xs), 2)]
    return xs[0]


def _permute_cols(w_ref, r0):
    lane = jax.lax.broadcasted_iota(jnp.int32, (PCH, 128), 1)
    e, c, hh, f = lane // 64, (lane % 64) // 8, (lane % 8) // 2, lane % 2
    idx = hh * 32 + 4 * c + 2 * e + f
    for m in range(3):
        v = [jnp.take_along_axis(w_ref[pl.ds(r0, PCH), m * M + g * 128:m * M + (g + 1) * 128], idx, axis=1)
             for g in range(NC)]
        for b in (1, 2, 4):
            hi = (c & b) != 0
            nv = list(v)
            for g in range(NC):
                if g & b == 0:
                    nv[g] = jnp.where(hi, pltpu.roll(v[g + b], 8 * b, 1), v[g])
                    nv[g + b] = jnp.where(hi, v[g + b], pltpu.roll(v[g], 128 - 8 * b, 1))
            v = nv
        for g in range(NC):
            w_ref[pl.ds(r0, PCH), m * M + g * 128:m * M + (g + 1) * 128] = v[g]


def _head_weight(w_ref, h):
    w32 = w_ref[h // 2]
    sh = jnp.asarray((1 - h % 2) * 16, jnp.int32).astype(U32)
    bits = (w32 << sh) & jnp.uint32(0xFFFF0000)
    return jax.lax.bitcast_convert_type(bits, F32).astype(BF16)


def _kernel(x_hbm, c_hbm, wq_hbm, wuk_hbm, wuv_hbm, wo_hbm, wqkv_hbm, wob_hbm, gw_ref, out_hbm,
            x_ref, c_ref, wq_ref, wuk_ref, wuv_ref, wo_ref, wqkv_ref, wob_ref,
            ctx_ref, kb_ref, vb_ref, qs_ref, ps_ref, ob_ref, k_ref, v_ref, o_ref, sems, wsem, osem):

    wqkv32 = wqkv_hbm.bitcast(U32)
    first, rest = pl.ds(0, 2 * PCH), pl.ds(2 * PCH, M // 2 - 2 * PCH)
    c_copy = pltpu.make_async_copy(c_hbm, c_ref, sems.at[0])
    x_copy = pltpu.make_async_copy(x_hbm, x_ref, sems.at[1])
    wo_copy = pltpu.make_async_copy(wo_hbm, wo_ref, sems.at[2])
    wqkv_first_copy = pltpu.make_async_copy(wqkv32.at[first], wqkv_ref.at[first], sems.at[3])
    wqkv_rest_copy = pltpu.make_async_copy(wqkv32.at[rest], wqkv_ref.at[rest], sems.at[4])

    def w_copies(j):
        return [pltpu.make_async_copy(src.bitcast(U32).at[:, j, :], dst.at[j], wsem.at[j])
                for src, dst in ((wuk_hbm, wuk_ref), (wuv_hbm, wuv_ref), (wq_hbm, wq_ref))]

    def wob_copies():
        return [pltpu.make_async_copy(wob_hbm.bitcast(U32).at[:, j, :], wob_ref.at[pl.ds(j * 32, 32), :], sems.at[5])
                for j in range(16)]

    def kv_proj(h):
        k_ref[h % 2] = _dot(c_ref[...], _head_weight(wuk_ref, h)).astype(BF16)
        v_ref[h % 2] = _dot(c_ref[...], _head_weight(wuv_ref, h)).astype(BF16)

    def head_step(h, last):
        _permute_cols(wqkv_ref, pl.multiple_of(h * PCH, PCH))
        wq = _head_weight(wq_ref, h)
        k = k_ref.at[h % 2]
        v = v_ref.at[h % 2]
        row = jax.lax.broadcasted_iota(jnp.int32, (T, T), 0)
        col = jax.lax.broadcasted_iota(jnp.int32, (T, T), 1)
        tri = col <= row
        nb = BQ // T
        for qi in (ORDER_LAST if last else ORDER):
            lo, hi = qi * BQ, (qi + 1) * BQ
            qb = (_dot(x_ref[lo:hi, :], wq) * (D ** -0.5 * LOG2E)).astype(BF16)
            sc = [_dot_nt(qb, k[0:lo + T, :])]
            sc += [_dot_nt(qb[j * T:], k[lo + j * T:lo + (j + 1) * T, :]) for j in range(1, nb)]
            pr, rl = [], []
            for r in range(nb):
                rows = slice(r * T, (r + 1) * T)
                if r == 0:
                    pieces = ([sc[0][rows, :lo]] if lo else []) + [jnp.where(tri, sc[0][rows, lo:], NEG)]
                else:
                    pieces = [sc[0][rows]] + [sc[j][(r - j) * T:(r - j + 1) * T] for j in range(1, r)]
                    pieces.append(jnp.where(tri, sc[r][:T], NEG))
                m = _tree(jnp.maximum, [jnp.max(t, axis=1, keepdims=True) for t in pieces])
                ps = [jnp.exp2(t - m) for t in pieces]
                rl.append(_recip(_tree(jnp.add, [jnp.sum(t, axis=1, keepdims=True) for t in ps])))
                if r == 0 and lo:
                    ps = [jnp.concatenate(ps, axis=1)]
                pr.append([t.astype(BF16) for t in ps])
            o = _dot(jnp.concatenate([pr[r][0] for r in range(nb)], axis=0), v[0:lo + T, :])
            os_ = [o[r * T:(r + 1) * T] for r in range(nb)]
            for j in range(1, nb):
                oj = _dot(jnp.concatenate([pr[r][j] for r in range(j, nb)], axis=0), v[lo + j * T:lo + (j + 1) * T, :])
                for r in range(j, nb):
                    os_[r] = os_[r] + oj[(r - j) * T:(r - j + 1) * T]
            for r in range(nb):
                ctx_ref[h, lo + r * T:lo + (r + 1) * T, :] = (os_[r] * rl[r]).astype(BF16)
        if not last:
            kv_proj(h + 1)

    c_copy.start()
    for c_ in w_copies(0):
        c_.start()
    x_copy.start()
    wqkv_first_copy.start()
    c_copy.wait()
    for c_ in w_copies(0):
        c_.wait()
    for c_ in w_copies(1):
        c_.start()
    kv_proj(0)
    x_copy.wait()
    wqkv_first_copy.wait()
    wqkv_rest_copy.start()

    @pl.loop(0, H - 1)
    def _(i):
        head_step(i, False)

        @pl.when(jnp.logical_and(i < H - 2, i % 2 == 0))
        def _():
            for c_ in w_copies(i // 2 + 1):
                c_.wait()

            @pl.when(i < H - 4)
            def _():
                for c_ in w_copies(i // 2 + 2):
                    c_.start()

        @pl.when(i == 1)
        def _():
            wqkv_rest_copy.wait()

        @pl.when(i == 2)
        def _():
            wo_copy.start()

        @pl.when(i == 4)
        def _():
            for c_ in wob_copies():
                c_.start()

    head_step(H - 1, True)

    kb_ref[:, RB:RB + HALO, :] = jnp.zeros((NC, HALO, 128), F32)
    vb_ref[:, RB:RB + HALO, :] = jnp.zeros((NC, HALO, 128), F32)
    wo_copy.wait()
    for c_ in wob_copies():
        c_.wait()

    def out_copy(r):
        return pltpu.make_async_copy(o_ref.at[r % 2], out_hbm.at[pl.ds(r * RB, RB), :], osem.at[r % 2])

    @pl.loop(0, NR)
    def _(r):
        @pl.when(r >= 2)
        def _():
            out_copy(r - 2).wait()
        kb_ref[:, 0:HALO, :] = kb_ref[:, RB:RB + HALO, :]
        vb_ref[:, 0:HALO, :] = vb_ref[:, RB:RB + HALO, :]
        r0 = pl.multiple_of(r * RB, RB)
        xb = x_ref[pl.ds(r0, RB), :]

        def wcol(n):
            return pltpu.bitcast(wqkv_ref[:, n * 128:(n + 1) * 128], BF16)

        a = [None]

        def a_term(h):
            t = _dot(ctx_ref[h, pl.ds(r0, RB), :], wo_ref[h])
            a[0] = t if a[0] is None else a[0] + t

        for c in range(NC):
            qs_ref[c] = _dot(xb, wcol(c)) * (32 ** -0.5 * LOG2E)
            kb_ref[c, HALO:, :] = _dot(xb, wcol(NC + c))
        even = jax.lax.broadcasted_iota(jnp.int32, (CH, 128), 1) % 2 == 0
        grow = r * RB + jax.lax.broadcasted_iota(jnp.int32, (CH, 128), 0)
        nch = RB // CH
        for ch in range(nch):
            if ch % (nch // NC) == 0:
                c = ch // (nch // NC)
                vb_ref[c, HALO:, :] = _dot(xb, wcol(2 * NC + c))
            a_term(ch)
            lo = ch * CH
            q = [qs_ref[c, lo:lo + CH, :] for c in range(NC)]
            lg = []
            for w in range(W):
                st = HALO - 2 * w + lo
                t = _tree(jnp.add, [q[c] * kb_ref[c, st:st + CH, :] for c in range(NC)])
                t = t + pltpu.roll(t, 64, 1)
                t = t + jnp.where(even, pltpu.roll(t, 127, 1), pltpu.roll(t, 1, 1))
                if w > 0 and lo < HALO:
                    t = jnp.where(grow + lo >= 2 * w, t, NEG)
                lg.append(t)
            m = _tree(jnp.maximum, lg)
            p = [jnp.exp2(t - m) for t in lg]
            rl = _recip(_tree(jnp.add, p))
            for w in range(W):
                ps_ref[w, lo:lo + CH, :] = p[w] * rl
        for ch in range(nch):
            a_term(nch + ch)
            lo = ch * CH
            p = [ps_ref[w, lo:lo + CH, :] for w in range(W)]
            for c in range(NC):
                o = _tree(jnp.add, [p[w] * vb_ref[c, HALO - 2 * w + lo:HALO - 2 * w + lo + CH, :] for w in range(W)])
                ob_ref[lo:lo + CH, c * 128:(c + 1) * 128] = o.astype(BF16)
        b = _dot(ob_ref[...], pltpu.bitcast(wob_ref[...], BF16))
        gate = jax.nn.sigmoid(jnp.sum(xb.astype(F32) * gw_ref[...].astype(F32), axis=1, keepdims=True))
        o_ref[r % 2] = (gate * a[0] + (1.0 - gate) * b).astype(o_ref.dtype)
        out_copy(r).start()

    out_copy(NR - 2).wait()
    out_copy(NR - 1).wait()


@jax.jit
def pallas_gated_mix__compressed_kv_cla__sliding_local_dilated__prompt_kernel(
        A_x, A_c_kv, A_w_q, A_w_uk, A_w_uv, A_w_o, B_x, B_wqkv, B_wo, gate_w):
    del B_x
    any_spec = pl.BlockSpec(memory_space=pl.ANY)
    out = pl.pallas_call(
        _kernel,
        in_specs=[any_spec] * 8 + [pl.BlockSpec(memory_space=pltpu.VMEM)],
        out_specs=any_spec,
        out_shape=jax.ShapeDtypeStruct((S, M), BF16),
        scratch_shapes=[
            pltpu.VMEM((S, M), BF16),
            pltpu.VMEM((S, DC), BF16),
            pltpu.VMEM((H // 2, M, D), U32),
            pltpu.VMEM((H // 2, DC, D), U32),
            pltpu.VMEM((H // 2, DC, D), U32),
            pltpu.VMEM((H, D, M), BF16),
            pltpu.VMEM((M // 2, 3 * M), U32),
            pltpu.VMEM((M // 2, M), U32),
            pltpu.VMEM((H, S, D), BF16),
            pltpu.VMEM((NC, HALO + RB, 128), F32),
            pltpu.VMEM((NC, HALO + RB, 128), F32),
            pltpu.VMEM((NC, RB, 128), F32),
            pltpu.VMEM((W, RB, 128), F32),
            pltpu.VMEM((RB, M), BF16),
            pltpu.VMEM((2, S, D), BF16),
            pltpu.VMEM((2, S, D), BF16),
            pltpu.VMEM((2, RB, M), BF16),
            pltpu.SemaphoreType.DMA((6,)),
            pltpu.SemaphoreType.DMA((H // 2,)),
            pltpu.SemaphoreType.DMA((2,)),
        ],
        compiler_params=pltpu.CompilerParams(
            vmem_limit_bytes=120 * 1024 * 1024,
        ),
    )(A_x.reshape(S, M), A_c_kv.reshape(S, DC), A_w_q, A_w_uk, A_w_uv, A_w_o, B_wqkv,
      B_wo.reshape(32, M // 32, M), gate_w.reshape(1, M))
    return out.reshape(1, S, M)
```
